```python
import os as _os
_os.environ.setdefault("JAX_PLATFORMS", "cpu")
import jax
import jax.numpy as jnp

def _softmax(x, axis=-1):
    return jax.nn.softmax(x, axis=axis)
def _gelu(x):
    return jax.nn.gelu(x, approximate=True)
def _silu(x):
    return jax.nn.silu(x)
def _sigmoid(x):
    return jax.nn.sigmoid(x)
def _layernorm(x, axis=-1, eps=1e-5):
    m = jnp.mean(x, axis=axis, keepdims=True)
    v = jnp.var(x, axis=axis, keepdims=True)
    return (x - m) / jnp.sqrt(v + eps)
def _scatter_add(tgt, idx, src, axis=0):
    return tgt.at[idx].add(src)
def _segment_sum(src, seg, n):
    return jax.ops.segment_sum(src, seg, n)
class _Rng:
    def __init__(self, key):
        self._k = key
    def _next(self):
        self._k, sub = jax.random.split(self._k)
        return sub
    def normal(self, shape):
        return jax.random.normal(self._next(), shape, dtype=jnp.bfloat16)
    def randint(self, lo, hi, shape):
        return jax.random.randint(self._next(), shape, lo, hi, dtype=jnp.int32)
    def uniform(self, shape, lo=0.0, hi=1.0):
        return jax.random.uniform(self._next(), shape, jnp.bfloat16, lo, hi)
    def permutation(self, n):
        return jax.random.permutation(self._next(), n)


kernel_name = 'concat_heads__spectral_gfnet__mha_block__prompt'

def setup_inputs():
    _rng = _Rng(jax.random.key(int.from_bytes(__import__("os").urandom(4), "little")))
    _w = (lambda a: (lambda t: t.astype(jnp.bfloat16) if jnp.issubdtype(t.dtype, jnp.floating) else t)(jnp.asarray(a)))
    def _A_setup():
        B, S, D = 1, 2048, 576
        Df = D // 2 + 1
        return {
            "x": _w((lambda *s: _rng.normal(s) * 0.05)(B, S, D)),
            "w_r": _w((lambda *s: _rng.normal(s) * 0.05)(S, Df) * 0.02),
            "w_i": _w((lambda *s: _rng.normal(s) * 0.05)(S, Df) * 0.02),
        }
    _A_in = _A_setup()

    def _B_setup():
        B, S, D, H = 1, 2048, 576, 32
        return {
            "x": _w((lambda *s: _rng.normal(s) * 0.1)(B, S, D)),
            "wqkv": _w((lambda *s: _rng.normal(s) * 0.1)(D, 3 * D)),
            "wo": _w((lambda *s: _rng.normal(s) * 0.05)(D, D)),
        }
    _B_in = _B_setup()

    return {
        "A_x": _A_in["x"],
        "A_w_r": _A_in["w_r"],
        "A_w_i": _A_in["w_i"],
        "B_x": _B_in["x"],
        "B_wqkv": _B_in["wqkv"],
        "B_wo": _B_in["wo"],
    }

def reference(A_x, A_w_r, A_w_i, B_x, B_wqkv, B_wo):
    def _A_ref(x, w_r, w_i):
        B, S, D = x.shape
        X = (lambda x, axes=(-2,-1): jnp.fft.rfft2(x.astype(jnp.float32), axes=axes))(x, axes=(-2, -1))
        W = w_r + 1j * w_i
        X = X * W
        y = (lambda x, s, axes=(-2,-1): jnp.fft.irfft2(x, s=s, axes=axes).astype(jnp.bfloat16))(X, (S, D), axes=(-2, -1))
        return y

    def _B_ref(x, wqkv, wo):
        B, S, D = x.shape
        H = 32
        Dh = D // H
        qkv = (lambda x, *d: x.transpose(*d))((x @ wqkv).reshape(B, S, 3, H, Dh), 2, 0, 3, 1, 4)
        q, k, v = qkv[0], qkv[1], qkv[2]
        scores = jnp.einsum("bhqd,bhkd->bhqk", q, k) * (Dh ** -0.5)
        p = _softmax(scores, axis=-1)
        o = jnp.einsum("bhqk,bhkd->bhqd", p, v)
        return (lambda x, *d: x.transpose(*d))(o, 0, 2, 1, 3).reshape(B, S, D) @ wo

    a = _A_ref(A_x, A_w_r, A_w_i)
    b = _B_ref(B_x, B_wqkv, B_wo)
    return jnp.concatenate([a, b], axis=-1)
```

```python
import numpy as np
import jax
import jax.numpy as jnp
from jax import lax
from jax.experimental import pallas as pl
from jax.experimental.pallas import tpu as pltpu

S = 2048
D = 576
H = 32
DH = 18
DF = D // 2 + 1
KP = 384
DP = 640
HPT = 7
NHT = 5
BQ = 512
CK = 128
UN = 2
UA = 1
UC = 1
UG = 1
NQ = S // BQ
NT = H * NQ
f32 = jnp.float32
bf16 = jnp.bfloat16
u32 = jnp.uint32


def _consts():
    d = np.arange(KP)[:, None]
    k = np.arange(KP)[None, :]
    ang = 2.0 * np.pi * ((d * k) % D) / D
    fc = np.cos(ang) * (d <= D // 2) * (k < DF)
    fc[D // 2] *= 0.5
    fs = -np.sin(ang) * (d < D // 2) * (k < DF)
    fd = np.stack([fc, fs])
    ck = np.where((d == 0) | (d == D // 2), 1.0, 2.0) * (d < DF) / D
    gd = np.stack([ck * np.cos(ang), -ck * np.sin(ang)])
    f1 = np.arange(16)[:, None, None]
    f2 = np.arange(128)[None, :, None]
    sl = np.arange(128)[None, None, :]
    a = 2.0 * np.pi * ((sl * (f1 + 16 * f2)) % S) / S
    mf = np.concatenate([np.cos(a), -np.sin(a)], axis=1)
    at = np.transpose(a, (0, 2, 1))
    mi = np.concatenate([np.cos(at), np.sin(at)], axis=1) / S
    c = lambda x: np.asarray(x, dtype=np.float32).astype(bf16)
    return c(np.concatenate([fd, gd])), c(np.concatenate([mf, mi]))


_FG, _MFI = _consts()


def _cadd(a, b):
    return (a[0] + b[0], a[1] + b[1])


def _csub(a, b):
    return (a[0] - b[0], a[1] - b[1])


def _fft4(a, b, c, d, inv):
    t0, t1, t2, t3 = _cadd(a, c), _csub(a, c), _cadd(b, d), _csub(b, d)
    if not inv:
        p = (t1[0] + t3[1], t1[1] - t3[0])
        m = (t1[0] - t3[1], t1[1] + t3[0])
    else:
        p = (t1[0] - t3[1], t1[1] + t3[0])
        m = (t1[0] + t3[1], t1[1] - t3[0])
    return [_cadd(t0, t2), p, _csub(t0, t2), m]


def _tw16(x, e, inv):
    e = e % 16
    if inv:
        e = (-e) % 16
    if e == 0:
        return x
    c = float(np.cos(2 * np.pi * e / 16))
    s = float(-np.sin(2 * np.pi * e / 16))
    re, im = x
    if e == 4:
        return (im, -re)
    if e == 12:
        return (-im, re)
    if e % 2 == 0:
        r = 0.7071067811865476
        sc, ss = np.sign(c), np.sign(s)
        nr = (re - im if ss / sc > 0 else re + im) * (r * sc)
        ni = (im + re if ss / sc > 0 else im - re) * (r * sc)
        return (nr, ni)
    return (re * c - im * s, re * s + im * c)


def _fft16(x, inv):
    a = [_fft4(x[n2], x[n2 + 4], x[n2 + 8], x[n2 + 12], inv) for n2 in range(4)]
    out = [None] * 16
    for k1 in range(4):
        col = [_tw16(a[n2][k1], n2 * k1, inv) for n2 in range(4)]
        r = _fft4(col[0], col[1], col[2], col[3], inv)
        for k2 in range(4):
            out[k1 + 4 * k2] = r[k2]
    return out


def _dot(a, b):
    return lax.dot_general(a, b, (((1,), (0,)), ((), ())), preferred_element_type=f32)


def _dot_tn(a, b):
    return lax.dot_general(a, b, (((0,), (0,)), ((), ())), preferred_element_type=f32)


def _for(n, unroll, body):
    if unroll >= n:
        for i in range(n):
            body(i)
    else:
        def b(i, c):
            for u in range(unroll):
                body(i * unroll + u)
            return c
        lax.fori_loop(0, n // unroll, b, 0)


def _aligned(x, m):
    return x if isinstance(x, int) else pl.multiple_of(x, m)


def _kernel(axt_h, wrt_h, wit_h, bxt_h, wqkv_h, wo_h, fg_h, mfi_h, out_h,
            axt_v, wrt_v, wit_v, bxt_v, wqkv_v, wo_v, fg_v, mfi_v,
            xf_v, u_v, wp_v, ya_v, wt_v, wk_v, wop_v, q32, k32, vth_v, s_v, qm_v, ot_v, ob_v,
            sem_c, sem_in, sem_out):
    def chunk_copy(src, dst, p, i):
        cols = pl.ds(_aligned(i * BQ, BQ), BQ)
        return pltpu.make_async_copy(src.at[:, cols], dst.at[:, cols], sem_c.at[p, i])

    chunked = [(bxt_h, bxt_v), (axt_h, axt_v), (wrt_h, wrt_v), (wit_h, wit_v)]
    c_wqkv = pltpu.make_async_copy(wqkv_h, wqkv_v, sem_in.at[0])
    c_fg = pltpu.make_async_copy(fg_h, fg_v, sem_in.at[1])
    c_mfi = pltpu.make_async_copy(mfi_h, mfi_v, sem_in.at[2])
    c_wo = pltpu.make_async_copy(wo_h, wo_v, sem_in.at[3])
    c_wqkv.start()
    for p, (a, b) in enumerate(chunked):
        chunk_copy(a, b, p, 0).start()
    c_wqkv.wait()
    for i in range(1, S // BQ):
        for p, (a, b) in enumerate(chunked):
            chunk_copy(a, b, p, i).start()
    c_fg.start()
    c_mfi.start()
    c_wo.start()

    w32 = wqkv_v.bitcast(u32)
    wk32 = wk_v.bitcast(u32)

    def repack(r0, nr, base):
        parts = []
        for t in range(NHT):
            lo = base + 126 * t
            n = min(126, base + D - lo)
            parts.append(w32[r0:r0 + nr, lo:lo + n])
            parts.append(jnp.zeros((nr, 128 - n), u32))
        return jnp.concatenate(parts, axis=1)

    wt_v[DP:DP + D, :] = wqkv_v[:, 2 * D:3 * D].T
    wq = jnp.concatenate([pltpu.bitcast(repack(r0, 96, 0), bf16) for r0 in range(0, D // 2, 96)], axis=0)
    wt_v[0:DP, :] = wq.T
    for r0 in range(0, D // 2, 96):
        wk32[r0:r0 + 96, :] = repack(r0, 96, D)

    qscale = float(DH ** -0.5 * np.log2(np.e))
    lane64 = lax.broadcasted_iota(jnp.int32, (64, 128), 1)
    ridx = (64 - lane64) & 127

    @pl.loop(0, S // BQ)
    def _(i):
        for p, (a, b) in enumerate(chunked):
            chunk_copy(a, b, p, i).wait()
        toks = pl.ds(pl.multiple_of(i * BQ, BQ), BQ)
        half = pl.ds(pl.multiple_of(i * (BQ // 2), BQ // 2), BQ // 2)
        xt = bxt_v[:, toks]
        qv = _dot(wt_v[...], xt)
        q = (qv[:DP] * qscale).astype(bf16)
        q32[:, :, toks] = pltpu.bitcast(q, u32).reshape(NHT, 64, BQ)
        v = qv[DP:]
        for h in range(H):
            vth_v[h, 0:16, toks] = v[18 * h:18 * h + 16]
            tail = jnp.concatenate([v[18 * h + 16:18 * h + 18], jnp.ones((1, BQ), f32), jnp.zeros((5, BQ), f32)], axis=0)
            vth_v[h, 16:24, toks] = tail
        kk = _dot_tn(xt, wk_v[...]).astype(bf16)
        kk = pltpu.bitcast(kk, u32)
        for t in range(NHT):
            k32[t, half, :] = kk[:, 128 * t:128 * t + 128]
        for p, w in enumerate((wrt_v, wit_v)):
            w2 = pltpu.bitcast(w[:, toks].T, u32)
            w2 = jnp.concatenate([w2, jnp.zeros((BQ // 2, KP - DF), u32)], axis=1)
            for c in range(3):
                wp_v[3 * p + c, half, :] = w2[:, 128 * c:128 * c + 128]
        for b in range(BQ // 128):
            x = axt_v[:, pl.ds(pl.multiple_of(i * BQ + b * 128, 128), 128)].T
            x32 = jnp.concatenate([pltpu.bitcast(x, u32), jnp.zeros((64, DP - D), u32)], axis=1)
            pm = [jnp.take_along_axis(x32[:, 128 * t:128 * t + 128], ridx, axis=1) for t in range(1, 5)]
            r = jnp.concatenate([jnp.where(lane64 <= 64, pm[3 - t], pm[2 - t]) for t in range(3)], axis=1)
            r = pltpu.bitcast(r, bf16).astype(f32)
            xx = x[:, :KP].astype(f32)
            xf_v[i * (BQ // 128) + b] = jnp.concatenate([xx + r, xx - r], axis=1).astype(bf16)

    c_fg.wait()

    def stage_ab(jj):
        rows = pl.ds(_aligned(jj * 16, 16), 16)
        tr = _dot(xf_v[:, rows, 0:KP].reshape(256, KP), fg_v[0])
        ti = _dot(xf_v[:, rows, KP:2 * KP].reshape(256, KP), fg_v[1])
        for c in range(3):
            lanes = slice(128 * c, 128 * c + 128)
            ys = []
            for hf in range(2):
                vals = [(tr[16 * n + 8 * hf:16 * n + 8 * hf + 8, lanes], ti[16 * n + 8 * hf:16 * n + 8 * hf + 8, lanes])
                        for n in range(16)]
                ys.append(_fft16(vals, False))
            for f1 in range(16):
                for p in range(2):
                    u_v[f1, rows, KP * p + 128 * c:KP * p + 128 * c + 128] = jnp.concatenate(
                        [ys[0][f1][p], ys[1][f1][p]], axis=0).astype(bf16)

    _for(8, UA, stage_ab)
    c_mfi.wait()

    def stage_cde(fp):
        wr2 = jnp.concatenate([wp_v[c, pl.ds(fp, 128, stride=8), :] for c in range(3)], axis=1)
        wi2 = jnp.concatenate([wp_v[3 + c, pl.ds(fp, 128, stride=8), :] for c in range(3)], axis=1)
        for par in range(2):
            f1 = 2 * fp + par
            if par == 0:
                wr = pltpu.bitcast(wr2 << 16, f32)
                wi = pltpu.bitcast(wi2 << 16, f32)
            else:
                wr = pltpu.bitcast(wr2 & jnp.uint32(0xFFFF0000), f32)
                wi = pltpu.bitcast(wi2 & jnp.uint32(0xFFFF0000), f32)
            p = _dot(mfi_v[f1], u_v[f1])
            xr = p[:128, :KP] - p[128:, KP:]
            xi = p[128:, :KP] + p[:128, KP:]
            zr = xr * wr - xi * wi
            zi = xr * wi + xi * wr
            z = jnp.concatenate([zr, zi], axis=1).astype(bf16)
            p2 = _dot(mfi_v[16 + f1], z)
            vr = p2[:128, :KP] - p2[128:, KP:]
            vi = p2[128:, :KP] + p2[:128, KP:]
            u_v[f1] = jnp.concatenate([vr, vi], axis=1).astype(bf16)

    _for(8, UC, stage_cde)

    lane128 = lax.broadcasted_iota(jnp.int32, (128, 128), 1)
    ridx128 = (64 - lane128) & 127

    def stage_fg(jj):
        rows = pl.ds(_aligned(jj * 16, 16), 16)
        res = [[None] * 6 for _ in range(16)]
        for c in range(3):
            vals = []
            for f1 in range(16):
                vals.append((u_v[f1, rows, 128 * c:128 * c + 128].astype(f32),
                             u_v[f1, rows, KP + 128 * c:KP + 128 * c + 128].astype(f32)))
            y = _fft16(vals, True)
            for n in range(16):
                res[n][c] = y[n][0].astype(bf16)
                res[n][3 + c] = y[n][1].astype(bf16)
        lr = jnp.concatenate([jnp.concatenate(r[:3], axis=1) for r in res], axis=0)
        li = jnp.concatenate([jnp.concatenate(r[3:], axis=1) for r in res], axis=0)
        e = _dot(lr, fg_v[2])
        o = _dot(li, fg_v[3])
        ya_v[:, rows, 0:KP] = (e + o).astype(bf16).reshape(16, 16, KP)
        dm = pltpu.bitcast((e[:, :256] - o[:, :256]).astype(bf16), u32)
        p0 = jnp.take_along_axis(dm[:, 0:128], ridx128, axis=1)
        p1 = jnp.take_along_axis(dm[:, 128:256], ridx128, axis=1)
        t3 = jnp.where(lane128 <= 64, p1, p0)
        t4 = jnp.where(lane128 < 64, p0, jnp.uint32(0))
        ya_v[:, rows, KP:DP] = pltpu.bitcast(jnp.concatenate([t3, t4], axis=1), bf16).reshape(16, 16, 256)

    _for(8, UG, stage_fg)

    ya2 = ya_v.reshape(S, DP)
    c_outa = pltpu.make_async_copy(ya2.at[:, pl.ds(0, 512)], out_h.at[:, pl.ds(0, 512)], sem_out.at[0])
    c_outa.start()

    rowq = lax.broadcasted_iota(jnp.int32, (64, BQ), 0)

    def idx(t):
        h = t // NQ
        return h, pl.ds(_aligned((t % NQ) * BQ, BQ), BQ)

    def prep_q(t, slot):
        h, qs = idx(t)
        ht = h // HPT
        j = h - ht * HPT
        m = (rowq >= 9 * j) & (rowq < 9 * j + 9)
        qm_v[slot] = jnp.where(m, q32[ht, :, qs], jnp.uint32(0))

    def qk_chunk(t, j, slot, m):
        h, _ = idx(t)
        kk = pltpu.bitcast(k32[h // HPT, j * CK // 2:(j + 1) * CK // 2, :], bf16)
        s = _dot(kk, pltpu.bitcast(qm_v[slot], bf16))
        s_v[slot, j * CK:(j + 1) * CK, :] = s
        mm = jnp.max(s.reshape(CK // 8, 8, BQ), axis=0)
        return mm if m is None else jnp.maximum(m, mm)

    def pv_chunk(t, j, slot, m, acc):
        h, _ = idx(t)
        s = s_v[slot, j * CK:(j + 1) * CK, :]
        p = jnp.exp2(s.reshape(CK // 8, 8, BQ) - m[None]).reshape(CK, BQ).astype(bf16)
        o = _dot(vth_v[h, :, j * CK:(j + 1) * CK], p)
        return o if acc is None else acc + o

    def fin_m(m):
        return jnp.broadcast_to(jnp.max(m, axis=0, keepdims=True), (8, BQ))

    def fin_o(t, acc):
        h, qs = idx(t)
        ot_v[h, :, qs] = acc * (1.0 / acc[18:19, :])

    NC = S // CK
    prep_q(0, 0)
    m = None
    for j in range(NC):
        m = qk_chunk(0, j, 0, m)
    m0 = fin_m(m)

    def body(it, m_cur):
        for u in range(UN):
            t = it * UN + u
            slot = u % 2
            tn = jnp.minimum(t + 1, NT - 1)
            prep_q(tn, 1 - slot)
            m = None
            acc = None
            for j in range(NC):
                m = qk_chunk(tn, j, 1 - slot, m)
                acc = pv_chunk(t, j, slot, m_cur, acc)
            fin_o(t, acc)
            m_cur = fin_m(m)
        return m_cur

    lax.fori_loop(0, NT // UN, body, m0)

    c_wo.wait()
    wop_v[:, 0:64] = jnp.zeros((D, 64), bf16)
    wop_v[:, 64:DP] = wo_v[...]
    OC = 512
    for i in range(S // OC):
        toks = pl.ds(i * OC, OC)
        o = jnp.concatenate([ot_v[h, 0:DH, toks] for h in range(H)], axis=0).astype(bf16)
        ob = _dot_tn(o, wop_v[...])
        first = ob[:, 0:128] + ya2[toks, 512:DP].astype(f32)
        ob_v[toks, 0:128] = first.astype(bf16)
        ob_v[toks, 128:DP] = ob[:, 128:].astype(bf16)
        pltpu.make_async_copy(ob_v.at[toks, :], out_h.at[toks, pl.ds(512, DP)], sem_out.at[1 + i]).start()
    c_outa.wait()
    for i in range(S // OC):
        toks = pl.ds(i * OC, OC)
        pltpu.make_async_copy(ob_v.at[toks, :], out_h.at[toks, pl.ds(512, DP)], sem_out.at[1 + i]).wait()


@jax.jit
def pallas_concat_heads__spectral_gfnet__mha_block__prompt_kernel(A_x, A_w_r, A_w_i, B_x, B_wqkv, B_wo):
    hbm = pl.BlockSpec(memory_space=pltpu.MemorySpace.HBM)
    V = pltpu.VMEM
    scratch = [
        V((D, S), bf16), V((DF, S), bf16), V((DF, S), bf16), V((D, S), bf16), V((D, 3 * D), bf16),
        V((D, D), bf16), V((4, KP, KP), bf16), V((32, 256, 128), bf16),
        V((16, 128, 2 * KP), bf16),
        V((16, 128, 2 * KP), bf16),
        V((6, S // 2, 128), u32),
        V((16, 128, DP), bf16),
        V((DP + D, D), bf16),
        V((D, DP), bf16),
        V((D, DP), bf16),
        V((NHT, 64, S), u32),
        V((NHT, S // 2, 128), u32),
        V((H, 24, S), f32),
        V((2, S, BQ), f32),
        V((2, 64, BQ), u32),
        V((H, 24, S), f32),
        V((S, DP), bf16),
        pltpu.SemaphoreType.DMA((4, 4)), pltpu.SemaphoreType.DMA((4,)), pltpu.SemaphoreType.DMA((5,)),
    ]
    args = (A_x[0].T, A_w_r.T, A_w_i.T, B_x[0].T, B_wqkv, B_wo, jnp.asarray(_FG), jnp.asarray(_MFI))
    args = [pltpu.with_memory_space_constraint(a, pltpu.MemorySpace.HBM) for a in args]
    out = pl.pallas_call(
        _kernel,
        out_shape=jax.ShapeDtypeStruct((S, 2 * D), bf16),
        in_specs=[hbm] * 8,
        out_specs=hbm,
        scratch_shapes=scratch,
        compiler_params=pltpu.CompilerParams(vmem_limit_bytes=110 * 1024 * 1024),
        name="fused",
    )(*args)
    return out.reshape(1, S, 2 * D)
```

```python
import numpy as np
import jax
import jax.numpy as jnp
from jax import lax
from jax.experimental import pallas as pl
from jax.experimental.pallas import tpu as pltpu

S = 2048
D = 576
H = 32
DH = 18
DF = D // 2 + 1
KP = 384
DP = 640
HPT = 7
NHT = 5
BQ = 512
CK = 128
UN = 8
SKA = 0
SKC = 2
SKG = 0
PEEL = 1
OC = 256
OA = 1
OE = 1
OG = 2
NQ = S // BQ
NT = H * NQ
f32 = jnp.float32
bf16 = jnp.bfloat16
u32 = jnp.uint32


def _consts():
    d = np.arange(KP)[:, None]
    k = np.arange(KP)[None, :]
    ang = 2.0 * np.pi * ((d * k) % D) / D
    fc = np.cos(ang) * (d <= D // 2) * (k < DF)
    fc[D // 2] *= 0.5
    fs = -np.sin(ang) * (d < D // 2) * (k < DF)
    fd = np.stack([fc, fs])
    ck = np.where((d == 0) | (d == D // 2), 1.0, 2.0) * (d < DF) / D
    gd = np.stack([ck * np.cos(ang), -ck * np.sin(ang)])
    f1 = np.arange(16)[:, None, None]
    f2 = np.arange(128)[None, :, None]
    sl = np.arange(128)[None, None, :]
    a = 2.0 * np.pi * ((sl * (f1 + 16 * f2)) % S) / S
    mf = np.concatenate([np.cos(a), -np.sin(a)], axis=1)
    at = np.transpose(a, (0, 2, 1))
    mi = np.concatenate([np.cos(at), np.sin(at)], axis=1) / S
    c = lambda x: np.asarray(x, dtype=np.float32).astype(bf16)
    return c(np.concatenate([fd, gd])), c(np.concatenate([mf, mi]))


_FG, _MFI = _consts()


def _cadd(a, b):
    return (a[0] + b[0], a[1] + b[1])


def _csub(a, b):
    return (a[0] - b[0], a[1] - b[1])


def _fft4(a, b, c, d, inv):
    t0, t1, t2, t3 = _cadd(a, c), _csub(a, c), _cadd(b, d), _csub(b, d)
    if not inv:
        p = (t1[0] + t3[1], t1[1] - t3[0])
        m = (t1[0] - t3[1], t1[1] + t3[0])
    else:
        p = (t1[0] - t3[1], t1[1] + t3[0])
        m = (t1[0] + t3[1], t1[1] - t3[0])
    return [_cadd(t0, t2), p, _csub(t0, t2), m]


def _tw16(x, e, inv):
    e = e % 16
    if inv:
        e = (-e) % 16
    if e == 0:
        return x
    c = float(np.cos(2 * np.pi * e / 16))
    s = float(-np.sin(2 * np.pi * e / 16))
    re, im = x
    if e == 4:
        return (im, -re)
    if e == 12:
        return (-im, re)
    if e % 2 == 0:
        r = 0.7071067811865476
        sc, ss = np.sign(c), np.sign(s)
        nr = (re - im if ss / sc > 0 else re + im) * (r * sc)
        ni = (im + re if ss / sc > 0 else im - re) * (r * sc)
        return (nr, ni)
    return (re * c - im * s, re * s + im * c)


def _fft16(x, inv):
    a = [_fft4(x[n2], x[n2 + 4], x[n2 + 8], x[n2 + 12], inv) for n2 in range(4)]
    out = [None] * 16
    for k1 in range(4):
        col = [_tw16(a[n2][k1], n2 * k1, inv) for n2 in range(4)]
        r = _fft4(col[0], col[1], col[2], col[3], inv)
        for k2 in range(4):
            out[k1 + 4 * k2] = r[k2]
    return out


def _dot(a, b):
    return lax.dot_general(a, b, (((1,), (0,)), ((), ())), preferred_element_type=f32)


def _dot_tn(a, b):
    return lax.dot_general(a, b, (((0,), (0,)), ((), ())), preferred_element_type=f32)


def _pipeline(total, skew, first, second, outer=1):
    n = total // outer

    def run(base):
        pend = {}
        for i in range(n + skew):
            if i < n:
                pend[i] = first(base, i)
            if i >= skew:
                second(base, i - skew, *pend.pop(i - skew))

    if outer == 1:
        run(0)
    else:
        pl.loop(0, outer)(lambda o: run(o * n))


def _aligned(x, m):
    return x if isinstance(x, int) else pl.multiple_of(x, m)


def _kernel(axt_h, wrt_h, wit_h, bxt_h, wqkv_h, wo_h, fg_h, mfi_h, out_h,
            axt_v, wrt_v, wit_v, bxt_v, wqkv_v, wo_v, fg_v, mfi_v,
            xf_v, u_v, wp_v, ya_v, wt_v, wop_v, q32, k32, vth_v, s_v, ot_v, ob_v,
            sem_c, sem_in, sem_out):
    def chunk_copy(src, dst, p, i):
        cols = pl.ds(_aligned(i * BQ, BQ), BQ)
        return pltpu.make_async_copy(src.at[:, cols], dst.at[:, cols], sem_c.at[p, i])

    chunked = [(bxt_h, bxt_v), (axt_h, axt_v), (wrt_h, wrt_v), (wit_h, wit_v)]
    c_fg = pltpu.make_async_copy(fg_h, fg_v, sem_in.at[0])
    c_mfi = pltpu.make_async_copy(mfi_h, mfi_v, sem_in.at[1])
    c_wo = pltpu.make_async_copy(wo_h, wo_v, sem_in.at[2])
    wparts = dict(v=(2 * D, D), q=(0, DP), k=(DP, 2 * D - DP))
    c_w = {n: pltpu.make_async_copy(wqkv_h.at[:, pl.ds(c0, nc)], wqkv_v.at[:, pl.ds(c0, nc)], sem_in.at[3 + i])
           for i, (n, (c0, nc)) in enumerate(wparts.items())}

    def w_ready(n):
        c0, nc = wparts[n]
        c_w[n].wait()
        wt_v[c0:c0 + nc, :] = wqkv_v[:, c0:c0 + nc].T

    qscale = float(DH ** -0.5 * np.log2(np.e))
    lane64 = lax.broadcasted_iota(jnp.int32, (64, 128), 1)
    ridx = (64 - lane64) & 127
    rowq = lax.broadcasted_iota(jnp.int32, (64, BQ), 0)

    def head_tiles(a):
        a = jnp.concatenate([a, jnp.zeros((DP - D, a.shape[1]), a.dtype)], axis=0)
        return [a[126 * t:126 * t + 128] for t in range(NHT)]

    def proj_v(toks, v):
        for h in range(H):
            vth_v[h, 0:16, toks] = v[18 * h:18 * h + 16]
            tail = jnp.concatenate([v[18 * h + 16:18 * h + 18], jnp.ones((1, BQ), f32), jnp.zeros((5, BQ), f32)], axis=0)
            vth_v[h, 16:24, toks] = tail

    def proj_q(toks, q_all):
        for t, q in enumerate(head_tiles(q_all * qscale)):
            qp = pltpu.bitcast(q.astype(bf16), u32)
            for j in range(min(HPT, H - HPT * t)):
                q32[HPT * t + j, :, toks] = jnp.where((rowq >= 9 * j) & (rowq < 9 * j + 9), qp, jnp.uint32(0))

    def proj_k(half, k_all):
        for t, k in enumerate(head_tiles(k_all)):
            k32[t, half, :] = pltpu.bitcast(k.astype(bf16).T, u32)

    def fft_prepass(i, toks, half):
        for p, w in enumerate((wrt_v, wit_v)):
            w2 = pltpu.bitcast(w[:, toks].T, u32)
            w2 = jnp.concatenate([w2, jnp.zeros((BQ // 2, KP - DF), u32)], axis=1)
            for c in range(3):
                wp_v[3 * p + c, half, :] = w2[:, 128 * c:128 * c + 128]
        for b in range(BQ // 128):
            x = axt_v[:, pl.ds(_aligned(i * BQ + b * 128, 128), 128)].T
            x32 = jnp.concatenate([pltpu.bitcast(x, u32), jnp.zeros((64, DP - D), u32)], axis=1)
            pm = [jnp.take_along_axis(x32[:, 128 * t:128 * t + 128], ridx, axis=1) for t in range(1, 5)]
            r = jnp.concatenate([jnp.where(lane64 <= 64, pm[3 - t], pm[2 - t]) for t in range(3)], axis=1)
            r = pltpu.bitcast(r, bf16).astype(f32)
            xx = x[:, :KP].astype(f32)
            xf_v[i * (BQ // 128) + b] = jnp.concatenate([xx + r, xx - r], axis=1).astype(bf16)

    toks0, half0 = pl.ds(0, BQ), pl.ds(0, BQ // 2)
    c_w["v"].start()
    chunk_copy(bxt_h, bxt_v, 0, 0).start()
    w_ready("v")
    chunk_copy(bxt_h, bxt_v, 0, 0).wait()
    c_w["q"].start()
    xt0 = bxt_v[:, toks0]
    proj_v(toks0, _dot(wt_v[2 * D:3 * D, :], xt0))
    c_w["k"].start()
    for p in range(1, 4):
        chunk_copy(*chunked[p], p, 0).start()
    w_ready("q")
    proj_q(toks0, _dot(wt_v[0:D, :], xt0))
    for i in range(1, S // BQ):
        for p, (a, b) in enumerate(chunked):
            chunk_copy(a, b, p, i).start()
    c_fg.start()
    c_mfi.start()
    c_wo.start()
    for p in range(1, 4):
        chunk_copy(*chunked[p], p, 0).wait()
    w_ready("k")
    proj_k(half0, _dot(wt_v[D:2 * D, :], xt0))
    fft_prepass(0, toks0, half0)

    @pl.loop(1, S // BQ)
    def _(i):
        for p, (a, b) in enumerate(chunked):
            chunk_copy(a, b, p, i).wait()
        toks = pl.ds(pl.multiple_of(i * BQ, BQ), BQ)
        half = pl.ds(pl.multiple_of(i * (BQ // 2), BQ // 2), BQ // 2)
        qkv = _dot(wt_v[...], bxt_v[:, toks])
        proj_q(toks, qkv[:D])
        proj_k(half, qkv[D:2 * D])
        proj_v(toks, qkv[2 * D:])
        fft_prepass(i, toks, half)

    c_fg.wait()

    def stage_a(base, jj):
        rows = pl.ds(_aligned((base + jj) * 16, 16), 16)
        tr = _dot(xf_v[:, rows, 0:KP].reshape(256, KP), fg_v[0])
        ti = _dot(xf_v[:, rows, KP:2 * KP].reshape(256, KP), fg_v[1])
        return tr, ti

    def stage_b(base, jj, tr, ti):
        rows = pl.ds(_aligned((base + jj) * 16, 16), 16)
        for c in range(3):
            lanes = slice(128 * c, 128 * c + 128)
            ys = []
            for hf in range(2):
                vals = [(tr[16 * n + 8 * hf:16 * n + 8 * hf + 8, lanes], ti[16 * n + 8 * hf:16 * n + 8 * hf + 8, lanes])
                        for n in range(16)]
                ys.append(_fft16(vals, False))
            for f1 in range(16):
                for p in range(2):
                    u_v[f1, rows, KP * p + 128 * c:KP * p + 128 * c + 128] = jnp.concatenate(
                        [ys[0][f1][p], ys[1][f1][p]], axis=0).astype(bf16)

    _pipeline(8, SKA, stage_a, stage_b, OA)
    c_mfi.wait()
    c_wo.wait()
    wop_v[:, 0:64] = jnp.zeros((D, 64), bf16)
    wop_v[:, 64:DP] = wo_v[...]

    def stage_cd(base, i):
        f1, fp, par = base + i, base // 2 + i // 2, i % 2
        wr2 = jnp.concatenate([wp_v[c, pl.ds(fp, 128, stride=8), :] for c in range(3)], axis=1)
        wi2 = jnp.concatenate([wp_v[3 + c, pl.ds(fp, 128, stride=8), :] for c in range(3)], axis=1)
        if par == 0:
            wr = pltpu.bitcast(wr2 << 16, f32)
            wi = pltpu.bitcast(wi2 << 16, f32)
        else:
            wr = pltpu.bitcast(wr2 & jnp.uint32(0xFFFF0000), f32)
            wi = pltpu.bitcast(wi2 & jnp.uint32(0xFFFF0000), f32)
        p = _dot(mfi_v[f1], u_v[f1])
        xr = p[:128, :KP] - p[128:, KP:]
        xi = p[128:, :KP] + p[:128, KP:]
        zr = xr * wr - xi * wi
        zi = xr * wi + xi * wr
        return (jnp.concatenate([zr, zi], axis=1).astype(bf16),)

    def stage_e(base, i, z):
        f1 = base + i
        p2 = _dot(mfi_v[16 + f1], z)
        vr = p2[:128, :KP] - p2[128:, KP:]
        vi = p2[128:, :KP] + p2[:128, KP:]
        xf_v[f1] = jnp.concatenate([vr, vi], axis=1).astype(bf16)

    _pipeline(16, SKC, stage_cd, stage_e, OE)

    lane128 = lax.broadcasted_iota(jnp.int32, (128, 128), 1)
    ridx128 = (64 - lane128) & 127

    def stage_f(base, jj):
        rows = pl.ds(_aligned((base + jj) * 16, 16), 16)
        res = [[None] * 6 for _ in range(16)]
        for c in range(3):
            vals = []
            for f1 in range(16):
                vals.append((xf_v[f1, rows, 128 * c:128 * c + 128].astype(f32),
                             xf_v[f1, rows, KP + 128 * c:KP + 128 * c + 128].astype(f32)))
            y = _fft16(vals, True)
            for n in range(16):
                res[n][c] = y[n][0].astype(bf16)
                res[n][3 + c] = y[n][1].astype(bf16)
        lr = jnp.concatenate([jnp.concatenate(r[:3], axis=1) for r in res], axis=0)
        li = jnp.concatenate([jnp.concatenate(r[3:], axis=1) for r in res], axis=0)
        return lr, li

    def stage_g(base, jj, lr, li):
        rows = pl.ds(_aligned((base + jj) * 16, 16), 16)
        e = _dot(lr, fg_v[2])
        o = _dot(li, fg_v[3])
        ya_v[:, rows, 0:KP] = (e + o).astype(bf16).reshape(16, 16, KP)
        dm = pltpu.bitcast((e[:, :256] - o[:, :256]).astype(bf16), u32)
        p0 = jnp.take_along_axis(dm[:, 0:128], ridx128, axis=1)
        p1 = jnp.take_along_axis(dm[:, 128:256], ridx128, axis=1)
        t3 = jnp.where(lane128 <= 64, p1, p0)
        t4 = jnp.where(lane128 < 64, p0, jnp.uint32(0))
        ya_v[:, rows, KP:DP] = pltpu.bitcast(jnp.concatenate([t3, t4], axis=1), bf16).reshape(16, 16, 256)

    _pipeline(8, SKG, stage_f, stage_g, OG)

    ya2 = ya_v.reshape(S, DP)
    c_outa = pltpu.make_async_copy(ya2.at[:, pl.ds(0, 512)], out_h.at[:, pl.ds(0, 512)], sem_out.at[0])
    c_outa.start()


    def idx(t):
        h = t // NQ
        return h, pl.ds(_aligned((t % NQ) * BQ, BQ), BQ)

    def qk_chunk(t, j, slot, m):
        h, qs = idx(t)
        kk = pltpu.bitcast(k32[h // HPT, j * CK // 2:(j + 1) * CK // 2, :], bf16)
        s = _dot(kk, pltpu.bitcast(q32[h, :, qs], bf16))
        s_v[slot, j * CK:(j + 1) * CK, :] = s
        mm = jnp.max(s.reshape(CK // 8, 8, BQ), axis=0)
        return mm if m is None else jnp.maximum(m, mm)

    def pv_chunk(t, j, slot, m, acc):
        h, _ = idx(t)
        s = s_v[slot, j * CK:(j + 1) * CK, :]
        p = jnp.exp2(s.reshape(CK // 8, 8, BQ) - m[None]).reshape(CK, BQ).astype(bf16)
        o = _dot(vth_v[h, :, j * CK:(j + 1) * CK], p)
        return o if acc is None else acc + o

    def fin_m(m):
        return jnp.broadcast_to(jnp.max(m, axis=0, keepdims=True), (8, BQ))

    def fin_o(t, acc):
        h, qs = idx(t)
        ot_v[h, :, qs] = acc * (1.0 / acc[18:19, :])

    NC = S // CK
    m = None
    for j in range(NC):
        m = qk_chunk(0, j, 0, m)
    m0 = fin_m(m)

    def task(t, slot, m_cur, last=False):
        m = None
        acc = None
        for j in range(NC):
            if not last:
                m = qk_chunk(jnp.minimum(t + 1, NT - 1), j, 1 - slot, m)
            acc = pv_chunk(t, j, slot, m_cur, acc)
        fin_o(t, acc)
        return None if last else fin_m(m)

    def body(it, m_cur):
        for u in range(UN):
            m_cur = task(it * UN + u, u % 2, m_cur)
        return m_cur

    n_it = NT // UN - PEEL
    m_cur = lax.fori_loop(0, n_it, body, m0)
    for t in range(n_it * UN, NT):
        m_cur = task(t, t % 2, m_cur, last=(t == NT - 1))

    for i in range(S // OC):
        toks = pl.ds(i * OC, OC)
        o = jnp.concatenate([ot_v[h, 0:DH, toks] for h in range(H)], axis=0).astype(bf16)
        ob = _dot_tn(o, wop_v[...])
        first = ob[:, 0:128] + ya2[toks, 512:DP].astype(f32)
        ob_v[toks, 0:128] = first.astype(bf16)
        ob_v[toks, 128:DP] = ob[:, 128:].astype(bf16)
        pltpu.make_async_copy(ob_v.at[toks, :], out_h.at[toks, pl.ds(512, DP)], sem_out.at[1 + i]).start()
    c_outa.wait()
    for i in range(S // OC):
        toks = pl.ds(i * OC, OC)
        pltpu.make_async_copy(ob_v.at[toks, :], out_h.at[toks, pl.ds(512, DP)], sem_out.at[1 + i]).wait()


@jax.jit
def pallas_concat_heads__spectral_gfnet__mha_block__prompt_kernel(A_x, A_w_r, A_w_i, B_x, B_wqkv, B_wo):
    hbm = pl.BlockSpec(memory_space=pltpu.MemorySpace.HBM)
    V = pltpu.VMEM
    scratch = [
        V((D, S), bf16), V((DF, S), bf16), V((DF, S), bf16), V((D, S), bf16), V((D, 3 * D), bf16),
        V((D, D), bf16), V((4, KP, KP), bf16), V((32, 256, 128), bf16),
        V((16, 128, 2 * KP), bf16),
        V((16, 128, 2 * KP), bf16),
        V((6, S // 2, 128), u32),
        V((16, 128, DP), bf16),
        V((3 * D, D), bf16),
        V((D, DP), bf16),
        V((H, 64, S), u32),
        V((NHT, S // 2, 128), u32),
        V((H, 24, S), f32),
        V((2, S, BQ), f32),
        V((H, 24, S), f32),
        V((S, DP), bf16),
        pltpu.SemaphoreType.DMA((4, 4)), pltpu.SemaphoreType.DMA((6,)), pltpu.SemaphoreType.DMA((1 + S // OC,)),
    ]
    args = (A_x[0].T, A_w_r.T, A_w_i.T, B_x[0].T, B_wqkv, B_wo, jnp.asarray(_FG), jnp.asarray(_MFI))
    out = pl.pallas_call(
        _kernel,
        out_shape=jax.ShapeDtypeStruct((S, 2 * D), bf16),
        in_specs=[hbm] * 8,
        out_specs=hbm,
        scratch_shapes=scratch,
        compiler_params=pltpu.CompilerParams(vmem_limit_bytes=110 * 1024 * 1024),
        name="fused",
    )(*args)
    return out.reshape(1, S, 2 * D)
```
